```python
import os as _os
_os.environ.setdefault("JAX_PLATFORMS", "cpu")
import jax
import jax.numpy as jnp

def _softmax(x, axis=-1):
    return jax.nn.softmax(x, axis=axis)
def _gelu(x):
    return jax.nn.gelu(x, approximate=True)
def _silu(x):
    return jax.nn.silu(x)
def _sigmoid(x):
    return jax.nn.sigmoid(x)
def _layernorm(x, axis=-1, eps=1e-5):
    m = jnp.mean(x, axis=axis, keepdims=True)
    v = jnp.var(x, axis=axis, keepdims=True)
    return (x - m) / jnp.sqrt(v + eps)
def _scatter_add(tgt, idx, src, axis=0):
    return tgt.at[idx].add(src)
def _segment_sum(src, seg, n):
    return jax.ops.segment_sum(src, seg, n)
class _Rng:
    def __init__(self, key):
        self._k = key
    def _next(self):
        self._k, sub = jax.random.split(self._k)
        return sub
    def normal(self, shape):
        return jax.random.normal(self._next(), shape, dtype=jnp.bfloat16)
    def randint(self, lo, hi, shape):
        return jax.random.randint(self._next(), shape, lo, hi, dtype=jnp.int32)
    def uniform(self, shape, lo=0.0, hi=1.0):
        return jax.random.uniform(self._next(), shape, jnp.bfloat16, lo, hi)
    def permutation(self, n):
        return jax.random.permutation(self._next(), n)


kernel_name = 'gated_mix__ssm_conv_s5__glu_gated_geglu__prompt'

def setup_inputs():
    _rng = _Rng(jax.random.key(int.from_bytes(__import__("os").urandom(4), "little")))
    _w = (lambda a: (lambda t: t.astype(jnp.bfloat16) if jnp.issubdtype(t.dtype, jnp.floating) else t)(jnp.asarray(a)))
    def _A_setup():
        B, S, D = 1, 2048, 1024
        P = D
        Lambda_re = -0.5 * jnp.exp((lambda *s: _rng.normal(s) * 0.4)(P))
        Lambda_im = (lambda *s: _rng.normal(s) * 0.4)(P) * 1.0
        B_re = (lambda *s: _rng.normal(s) * 0.4)(P, D) * (D ** -0.5)
        B_im = (lambda *s: _rng.normal(s) * 0.4)(P, D) * (D ** -0.5)
        C_re = (lambda *s: _rng.normal(s) * 0.4)(D, P) * (P ** -0.5)
        C_im = (lambda *s: _rng.normal(s) * 0.4)(D, P) * (P ** -0.5)
        log_dt = (lambda *s: _rng.normal(s) * 0.4)(P) * 0.3 - 2.0
        Dskip = (lambda *s: _rng.normal(s) * 0.4)(D)
        return {
            "x": _w((lambda *s: _rng.normal(s) * 0.05)(B, S, D)),
            "Lambda_re": _w(Lambda_re),
            "Lambda_im": _w(Lambda_im),
            "B_re": _w(B_re),
            "B_im": _w(B_im),
            "C_re": _w(C_re),
            "C_im": _w(C_im),
            "log_dt": _w(log_dt),
            "Dskip": _w(Dskip),
        }
    _A_in = _A_setup()

    def _B_setup():
        B, S, Dm, Df = 1, 2048, 1024, 3584
        return {
            "x": _w((lambda *s: _rng.normal(s) * 0.05)(B, S, Dm)),
            "w_gate": _w((lambda *s: _rng.normal(s) * 1.6)(Dm, Df) * (Dm ** -0.5)),
            "w_up": _w((lambda *s: _rng.normal(s) * 1.6)(Dm, Df) * (Dm ** -0.5)),
            "w_down": _w((lambda *s: _rng.normal(s) * 1.6)(Df, Dm) * (Df ** -0.5)),
        }
    _B_in = _B_setup()

    return {
        "A_x": _A_in["x"],
        "A_Lambda_re": _A_in["Lambda_re"],
        "A_Lambda_im": _A_in["Lambda_im"],
        "A_B_re": _A_in["B_re"],
        "A_B_im": _A_in["B_im"],
        "A_C_re": _A_in["C_re"],
        "A_C_im": _A_in["C_im"],
        "A_log_dt": _A_in["log_dt"],
        "A_Dskip": _A_in["Dskip"],
        "B_x": _B_in["x"],
        "B_w_gate": _B_in["w_gate"],
        "B_w_up": _B_in["w_up"],
        "B_w_down": _B_in["w_down"],
        "gate_w": _w((lambda *s: _rng.normal(s) * 0.05)(1024) * 16.0),
    }

def reference(A_x, A_Lambda_re, A_Lambda_im, A_B_re, A_B_im, A_C_re, A_C_im, A_log_dt, A_Dskip, B_x, B_w_gate, B_w_up, B_w_down, gate_w):
    def _A_ref(x, Lambda_re, Lambda_im, B_re, B_im, C_re, C_im, log_dt, Dskip):
        Bsz, L, H = x.shape
        Lam = Lambda_re + 1j * Lambda_im
        Bmat = B_re + 1j * B_im
        Cmat = C_re + 1j * C_im
        dt = jnp.exp(log_dt)
        Lam_bar = jnp.exp(dt * Lam)
        B_bar = ((Lam_bar - 1.0) / Lam)[:, None] * Bmat
        Bu = jnp.einsum("bld,pd->blp", x + 0j, B_bar)
        h = jnp.zeros_like(Bu[:, 0, :])
        hs = []
        for t in range(L):
            h = Lam_bar[None, :] * h + Bu[:, t, :]
            hs.append(h)
        hseq = jnp.stack(hs, 1)
        y = 2.0 * jnp.einsum("blp,dp->bld", hseq, Cmat).real + x * Dskip[None, None, :]
        return y

    def _B_ref(x, w_gate, w_up, w_down):
        g = jnp.einsum("bsd,df->bsf", x, w_gate)
        u = jnp.einsum("bsd,df->bsf", x, w_up)
        h = _gelu(g) * u
        return jnp.einsum("bsf,fd->bsd", h, w_down)

    x = A_x
    g = _sigmoid((x * gate_w).sum(-1, keepdims=True))
    a = _A_ref(x, A_Lambda_re, A_Lambda_im, A_B_re, A_B_im, A_C_re, A_C_im, A_log_dt, A_Dskip)
    b = _B_ref(x, B_w_gate, B_w_up, B_w_down)
    return g * a + (1 - g) * b
```

```python
import functools

import jax
import jax.numpy as jnp
import jax.experimental.pallas as pl
import jax.experimental.pallas.tpu as pltpu

_NT = (((1,), (1,)), ((), ()))
_CB = 128
_NB0 = 2
_X1AT = 5


def _gelu_tanh(x):
    c = 0.7978845608028654
    return 0.5 * x * (1.0 + jnp.tanh(c * (x + 0.044715 * (x * x * x))))


def _kernel(x_hbm, lre_ref, lim_ref, ldt_ref, dsk_ref, gw_ref,
            bre_hbm, bim_hbm, cre_hbm, cim_hbm, wg_hbm, wu_hbm, wd_hbm,
            o_hbm,
            x_v, bre_v, bim_v, cre_v, cim_v, wg_v, wu_v, wd_v,
            xsems, osems, bsems, sems,
            tab, carry, hs, acc,
            *, nh, ts, tf, nf, P):
    nb = P // _CB
    ng = ts // 8

    def vec(ref):
        return ref[...].reshape(1, P).astype(jnp.float32)

    def x_copy(h):
        r0 = pl.multiple_of(h * ts, ts)
        return pltpu.make_async_copy(x_hbm.at[pl.ds(r0, ts), :], x_v.at[h], xsems.at[h])

    def o_copy(h):
        r0 = pl.multiple_of(h * ts, ts)
        return pltpu.make_async_copy(acc.at[h], o_hbm.at[pl.ds(r0, ts), :], osems.at[h])

    def b_copies(n):
        rs = pl.ds(n * _CB, _CB)
        return [pltpu.make_async_copy(bre_hbm.at[rs, :], bre_v.at[rs, :], bsems.at[2 * n]),
                pltpu.make_async_copy(bim_hbm.at[rs, :], bim_v.at[rs, :], bsems.at[2 * n + 1])]

    def c_copies():
        return [pltpu.make_async_copy(cre_hbm, cre_v, sems.at[0]),
                pltpu.make_async_copy(cim_hbm, cim_v, sems.at[1])]

    def f_copies(j):
        c0 = pl.multiple_of(j * tf, 128)
        return [pltpu.make_async_copy(wg_hbm.at[:, pl.ds(c0, tf)], wg_v.at[j], sems.at[2 + 3 * j]),
                pltpu.make_async_copy(wu_hbm.at[:, pl.ds(c0, tf)], wu_v.at[j], sems.at[3 + 3 * j]),
                pltpu.make_async_copy(wd_hbm.at[pl.ds(c0, tf), :], wd_v.at[j], sems.at[4 + 3 * j])]

    def init():
        x_copy(0).start()
        for n in range(_NB0):
            for cp in b_copies(n):
                cp.start()
        lre = vec(lre_ref)
        lim = vec(lim_ref)
        dt = jnp.exp(vec(ldt_ref)).astype(jnp.bfloat16).astype(jnp.float32)
        are = dt * lre
        aim = dt * lim
        mag = jnp.exp(are)
        nr = mag * jnp.cos(aim) - 1.0
        ni = mag * jnp.sin(aim)
        den = lre * lre + lim * lim
        cr = (nr * lre + ni * lim) / den
        ci = (ni * lre - nr * lim) / den
        row = jax.lax.broadcasted_iota(jnp.int32, (8, P), 0)
        tab[0] = jnp.broadcast_to(cr, (8, P))
        tab[1] = jnp.broadcast_to(ci, (8, P))
        for n, k in enumerate((1, 2, 4)):
            m = jnp.exp(k * are)
            pr = jnp.broadcast_to(m * jnp.cos(k * aim), (8, P))
            pi = jnp.broadcast_to(m * jnp.sin(k * aim), (8, P))
            tab[2 + 2 * n] = jnp.where(row >= k, pr, 0.0)
            tab[3 + 2 * n] = jnp.where(row >= k, pi, 0.0)
        kf = (row + 1).astype(jnp.float32)
        m = jnp.exp(kf * are)
        tab[8] = m * jnp.cos(kf * aim)
        tab[9] = m * jnp.sin(kf * aim)
        carry[...] = jnp.zeros_like(carry)

    def ssm_in(first, h):
        x = x_v[h]
        for n in range(nb):
            if first:
                for cp in b_copies(n):
                    cp.wait()
                if n + _NB0 < nb:
                    for cp in b_copies(n + _NB0):
                        cp.start()
                if n == _X1AT:
                    x_copy(1).start()
            cs = slice(n * _CB, (n + 1) * _CB)
            ur_all = jax.lax.dot_general(x, bre_v[cs, :], _NT, preferred_element_type=jnp.float32)
            ui_all = jax.lax.dot_general(x, bim_v[cs, :], _NT, preferred_element_type=jnp.float32)
            cfr = tab[0, :, cs]
            cfi = tab[1, :, cs]
            trs = [(tab[2 + 2 * k, :, cs], tab[3 + 2 * k, :, cs]) for k in range(3)]
            pr = tab[8, :, cs]
            pi = tab[9, :, cs]
            cr_ = carry[0:1, cs]
            ci_ = carry[1:2, cs]
            for g in range(ng):
                ur = ur_all[g * 8:(g + 1) * 8]
                ui = ui_all[g * 8:(g + 1) * 8]
                vr = cfr * ur - cfi * ui
                vi = cfr * ui + cfi * ur
                for k, (tr, ti) in zip((1, 2, 4), trs):
                    sr = pltpu.roll(vr, k, 0)
                    si = pltpu.roll(vi, k, 0)
                    vr, vi = vr + (tr * sr - ti * si), vi + (tr * si + ti * sr)
                cbr = jnp.broadcast_to(cr_, (8, _CB))
                cbi = jnp.broadcast_to(ci_, (8, _CB))
                vr = vr + (pr * cbr - pi * cbi)
                vi = vi + (pr * cbi + pi * cbr)
                hs[h, g * 8:(g + 1) * 8, n * _CB:(n + 1) * _CB] = vr
                hs[h, g * 8:(g + 1) * 8, P + n * _CB:P + (n + 1) * _CB] = vi
                cr_, ci_ = vr[7:8, :], vi[7:8, :]
            carry[0:1, cs] = cr_
            carry[1:2, cs] = ci_
        acc[h] = jnp.zeros(acc.shape[1:], acc.dtype)

    init()
    x_copy(0).wait()
    ssm_in(True, 0)

    def sbody(h, c):
        x_copy(h).wait()

        @pl.when(h + 1 < nh)
        def _():
            x_copy(h + 1).start()

        @pl.when(h == 1)
        def _():
            for cp in f_copies(0):
                cp.start()

        ssm_in(False, h)
        return c

    jax.lax.fori_loop(1, nh, sbody, 0)

    def fbody(it, c):
        j = it // nh
        h = it % nh

        @pl.when(h == 0)
        def _():
            for cp in f_copies(j):
                cp.wait()

            @pl.when(j + 1 < nf)
            def _():
                for cp in f_copies(j + 1):
                    cp.start()

            @pl.when(j + 1 == nf)
            def _():
                for cp in c_copies():
                    cp.start()

        xx = x_v[h]
        gj = jnp.dot(xx, wg_v[j], preferred_element_type=jnp.float32)
        uj = jnp.dot(xx, wu_v[j], preferred_element_type=jnp.float32)
        hj = (_gelu_tanh(gj) * uj).astype(jnp.bfloat16)
        acc[h] += jnp.dot(hj, wd_v[j], preferred_element_type=jnp.float32)
        return c

    jax.lax.fori_loop(0, nf * nh, fbody, 0)

    for cp in c_copies():
        cp.wait()

    def cbody(h, c):
        hr = hs[h, :, :P].astype(jnp.bfloat16)
        hi = hs[h, :, P:].astype(jnp.bfloat16)
        y = (jax.lax.dot_general(hr, cre_v[...], _NT, preferred_element_type=jnp.float32)
             - jax.lax.dot_general(hi, cim_v[...], _NT, preferred_element_type=jnp.float32))
        xf = x_v[h].astype(jnp.float32)
        ya = 2.0 * y + xf * vec(dsk_ref)
        gate = jax.nn.sigmoid(jnp.sum(xf * vec(gw_ref), axis=-1, keepdims=True))
        acc[h] = gate * ya + (1.0 - gate) * acc[h]
        o_copy(h).start()
        return c

    jax.lax.fori_loop(0, nh, cbody, 0)
    for h in range(nh):
        o_copy(h).wait()


@jax.jit
def pallas_gated_mix__ssm_conv_s5__glu_gated_geglu__prompt_kernel(
    A_x: jax.Array,
    A_Lambda_re: jax.Array,
    A_Lambda_im: jax.Array,
    A_B_re: jax.Array,
    A_B_im: jax.Array,
    A_C_re: jax.Array,
    A_C_im: jax.Array,
    A_log_dt: jax.Array,
    A_Dskip: jax.Array,
    B_x: jax.Array,
    B_w_gate: jax.Array,
    B_w_up: jax.Array,
    B_w_down: jax.Array,
    gate_w: jax.Array,
):
    Bsz, S, D = A_x.shape
    P = A_Lambda_re.shape[0]
    Df = B_w_gate.shape[1]
    ts = 256
    tf = 896
    nf = Df // tf
    nh = S // ts
    x2 = A_x.reshape(S, D)
    vec_spec = pl.BlockSpec((P,), lambda i: (0,))
    any_spec = pl.BlockSpec(memory_space=pl.ANY)
    out = pl.pallas_call(
        functools.partial(_kernel, nh=nh, ts=ts, tf=tf, nf=nf, P=P),
        grid=(1,),
        in_specs=[any_spec,
                  vec_spec, vec_spec, vec_spec, vec_spec, vec_spec,
                  any_spec, any_spec, any_spec, any_spec, any_spec, any_spec, any_spec],
        out_specs=any_spec,
        out_shape=jax.ShapeDtypeStruct((S, D), jnp.float32),
        scratch_shapes=[
            pltpu.VMEM((nh, ts, D), jnp.bfloat16),
            pltpu.VMEM((P, D), jnp.bfloat16),
            pltpu.VMEM((P, D), jnp.bfloat16),
            pltpu.VMEM((D, P), jnp.bfloat16),
            pltpu.VMEM((D, P), jnp.bfloat16),
            pltpu.VMEM((nf, D, tf), jnp.bfloat16),
            pltpu.VMEM((nf, D, tf), jnp.bfloat16),
            pltpu.VMEM((nf, tf, D), jnp.bfloat16),
            pltpu.SemaphoreType.DMA((nh,)),
            pltpu.SemaphoreType.DMA((nh,)),
            pltpu.SemaphoreType.DMA((2 * (P // _CB),)),
            pltpu.SemaphoreType.DMA((2 + 3 * nf,)),
            pltpu.VMEM((10, 8, P), jnp.float32),
            pltpu.VMEM((8, P), jnp.float32),
            pltpu.VMEM((nh, ts, 2 * P), jnp.float32),
            pltpu.VMEM((nh, ts, D), jnp.float32),
        ],
        compiler_params=pltpu.CompilerParams(
            dimension_semantics=("arbitrary",),
            vmem_limit_bytes=110 * 1024 * 1024,
        ),
    )(x2, A_Lambda_re, A_Lambda_im, A_log_dt, A_Dskip, gate_w,
      A_B_re, A_B_im, A_C_re, A_C_im, B_w_gate, B_w_up, B_w_down)
    return out.reshape(Bsz, S, D)
```

```python
import functools

import jax
import jax.numpy as jnp
import jax.experimental.pallas as pl
import jax.experimental.pallas.tpu as pltpu

_NT = (((1,), (1,)), ((), ()))
_CB = 128
_NB0 = 2
_X1AT = 5


def _gelu_tanh(x):
    c = 0.7978845608028654
    return 0.5 * x * (1.0 + jnp.tanh(c * (x + 0.044715 * (x * x * x))))


def _kernel(x_hbm, lre_ref, lim_ref, ldt_ref, dsk_ref, gw_ref,
            bre_hbm, bim_hbm, cre_hbm, cim_hbm, wg_hbm, wu_hbm, wd_hbm,
            o_hbm,
            x_v, bre_v, bim_v, cre_v, cim_v, wg_v, wu_v, wd_v,
            xsems, osems, bsems, sems,
            tab, carry, hs, acc,
            *, nh, ts, tf, nf, P):
    nb = P // _CB
    ng = ts // 8

    def vec(ref):
        return ref[...].reshape(1, P).astype(jnp.float32)

    def x_copy(h):
        r0 = pl.multiple_of(h * ts, ts)
        return pltpu.make_async_copy(x_hbm.at[pl.ds(r0, ts), :], x_v.at[h], xsems.at[h])

    def o_copy(h):
        r0 = pl.multiple_of(h * ts, ts)
        return pltpu.make_async_copy(acc.at[h], o_hbm.at[pl.ds(r0, ts), :], osems.at[h])

    def b_copies(n):
        rs = pl.ds(n * _CB, _CB)
        return [pltpu.make_async_copy(bre_hbm.at[rs, :], bre_v.at[rs, :], bsems.at[2 * n]),
                pltpu.make_async_copy(bim_hbm.at[rs, :], bim_v.at[rs, :], bsems.at[2 * n + 1])]

    def c_copies():
        return [pltpu.make_async_copy(cre_hbm, cre_v, sems.at[0]),
                pltpu.make_async_copy(cim_hbm, cim_v, sems.at[1])]

    def f_copies(j):
        c0 = pl.multiple_of(j * tf, 128)
        return [pltpu.make_async_copy(wg_hbm.at[:, pl.ds(c0, tf)], wg_v.at[j], sems.at[2 + 3 * j]),
                pltpu.make_async_copy(wu_hbm.at[:, pl.ds(c0, tf)], wu_v.at[j], sems.at[3 + 3 * j]),
                pltpu.make_async_copy(wd_hbm.at[pl.ds(c0, tf), :], wd_v.at[j], sems.at[4 + 3 * j])]

    def init():
        x_copy(0).start()
        for n in range(_NB0):
            for cp in b_copies(n):
                cp.start()
        lre = vec(lre_ref)
        lim = vec(lim_ref)
        dt = jnp.exp(vec(ldt_ref)).astype(jnp.bfloat16).astype(jnp.float32)
        are = dt * lre
        aim = dt * lim
        mag = jnp.exp(are)
        nr = mag * jnp.cos(aim) - 1.0
        ni = mag * jnp.sin(aim)
        den = lre * lre + lim * lim
        cr = (nr * lre + ni * lim) / den
        ci = (ni * lre - nr * lim) / den
        row = jax.lax.broadcasted_iota(jnp.int32, (8, P), 0)
        tab[0] = jnp.broadcast_to(cr, (8, P))
        tab[1] = jnp.broadcast_to(ci, (8, P))
        for n, k in enumerate((1, 2, 4)):
            m = jnp.exp(k * are)
            pr = jnp.broadcast_to(m * jnp.cos(k * aim), (8, P))
            pi = jnp.broadcast_to(m * jnp.sin(k * aim), (8, P))
            tab[2 + 2 * n] = jnp.where(row >= k, pr, 0.0)
            tab[3 + 2 * n] = jnp.where(row >= k, pi, 0.0)
        kf = (row + 1).astype(jnp.float32)
        m = jnp.exp(kf * are)
        tab[8] = m * jnp.cos(kf * aim)
        tab[9] = m * jnp.sin(kf * aim)
        carry[...] = jnp.zeros_like(carry)

    def ssm_in(first, h):
        x = x_v[h]
        for n in range(nb):
            if first:
                for cp in b_copies(n):
                    cp.wait()
                if n + _NB0 < nb:
                    for cp in b_copies(n + _NB0):
                        cp.start()
                if n == _X1AT:
                    x_copy(1).start()
            cs = slice(n * _CB, (n + 1) * _CB)
            ur_all = jax.lax.dot_general(x, bre_v[cs, :], _NT, preferred_element_type=jnp.float32)
            ui_all = jax.lax.dot_general(x, bim_v[cs, :], _NT, preferred_element_type=jnp.float32)
            cfr = tab[0, :, cs]
            cfi = tab[1, :, cs]
            trs = [(tab[2 + 2 * k, :, cs], tab[3 + 2 * k, :, cs]) for k in range(3)]
            pr = tab[8, :, cs]
            pi = tab[9, :, cs]
            cr_ = carry[0:1, cs]
            ci_ = carry[1:2, cs]
            for g in range(ng):
                ur = ur_all[g * 8:(g + 1) * 8]
                ui = ui_all[g * 8:(g + 1) * 8]
                vr = cfr * ur - cfi * ui
                vi = cfr * ui + cfi * ur
                for k, (tr, ti) in zip((1, 2, 4), trs):
                    sr = pltpu.roll(vr, k, 0)
                    si = pltpu.roll(vi, k, 0)
                    vr, vi = vr + (tr * sr - ti * si), vi + (tr * si + ti * sr)
                cbr = jnp.broadcast_to(cr_, (8, _CB))
                cbi = jnp.broadcast_to(ci_, (8, _CB))
                vr = vr + (pr * cbr - pi * cbi)
                vi = vi + (pr * cbi + pi * cbr)
                hs[h, g * 8:(g + 1) * 8, n * _CB:(n + 1) * _CB] = vr
                hs[h, g * 8:(g + 1) * 8, P + n * _CB:P + (n + 1) * _CB] = vi
                cr_, ci_ = vr[7:8, :], vi[7:8, :]
            carry[0:1, cs] = cr_
            carry[1:2, cs] = ci_
        acc[h] = jnp.zeros(acc.shape[1:], acc.dtype)

    init()
    x_copy(0).wait()
    ssm_in(True, 0)

    def sbody(h, c):
        x_copy(h).wait()

        @pl.when(h + 1 < nh)
        def _():
            x_copy(h + 1).start()

        @pl.when(h == 1)
        def _():
            for cp in f_copies(0):
                cp.start()

        ssm_in(False, h)
        return c

    jax.lax.fori_loop(1, nh, sbody, 0)

    def fbody(it, c):
        j = it // (nh // 2)
        h = it % (nh // 2)

        @pl.when(h == 0)
        def _():
            for cp in f_copies(j):
                cp.wait()

            @pl.when(j + 1 < nf)
            def _():
                for cp in f_copies(j + 1):
                    cp.start()

            @pl.when(j + 1 == nf)
            def _():
                for cp in c_copies():
                    cp.start()

        D = x_v.shape[-1]
        hsl = pl.ds(2 * h, 2)
        xx = x_v[hsl].reshape(2 * ts, D)
        gj = jnp.dot(xx, wg_v[j], preferred_element_type=jnp.float32)
        uj = jnp.dot(xx, wu_v[j], preferred_element_type=jnp.float32)
        hj = (_gelu_tanh(gj) * uj).astype(jnp.bfloat16)
        acc[hsl] += jnp.dot(hj, wd_v[j], preferred_element_type=jnp.float32).reshape(2, ts, D)
        return c

    jax.lax.fori_loop(0, nf * (nh // 2), fbody, 0)

    for cp in c_copies():
        cp.wait()

    def cbody(h, c):
        hr = hs[h, :, :P].astype(jnp.bfloat16)
        hi = hs[h, :, P:].astype(jnp.bfloat16)
        y = (jax.lax.dot_general(hr, cre_v[...], _NT, preferred_element_type=jnp.float32)
             - jax.lax.dot_general(hi, cim_v[...], _NT, preferred_element_type=jnp.float32))
        xf = x_v[h].astype(jnp.float32)
        ya = 2.0 * y + xf * vec(dsk_ref)
        gate = jax.nn.sigmoid(jnp.sum(xf * vec(gw_ref), axis=-1, keepdims=True))
        acc[h] = gate * ya + (1.0 - gate) * acc[h]
        o_copy(h).start()
        return c

    jax.lax.fori_loop(0, nh, cbody, 0)
    for h in range(nh):
        o_copy(h).wait()


@jax.jit
def pallas_gated_mix__ssm_conv_s5__glu_gated_geglu__prompt_kernel(
    A_x: jax.Array,
    A_Lambda_re: jax.Array,
    A_Lambda_im: jax.Array,
    A_B_re: jax.Array,
    A_B_im: jax.Array,
    A_C_re: jax.Array,
    A_C_im: jax.Array,
    A_log_dt: jax.Array,
    A_Dskip: jax.Array,
    B_x: jax.Array,
    B_w_gate: jax.Array,
    B_w_up: jax.Array,
    B_w_down: jax.Array,
    gate_w: jax.Array,
):
    Bsz, S, D = A_x.shape
    P = A_Lambda_re.shape[0]
    Df = B_w_gate.shape[1]
    ts = 256
    tf = 896
    nf = Df // tf
    nh = S // ts
    x2 = A_x.reshape(S, D)
    vec_spec = pl.BlockSpec((P,), lambda i: (0,))
    any_spec = pl.BlockSpec(memory_space=pl.ANY)
    out = pl.pallas_call(
        functools.partial(_kernel, nh=nh, ts=ts, tf=tf, nf=nf, P=P),
        grid=(1,),
        in_specs=[any_spec,
                  vec_spec, vec_spec, vec_spec, vec_spec, vec_spec,
                  any_spec, any_spec, any_spec, any_spec, any_spec, any_spec, any_spec],
        out_specs=any_spec,
        out_shape=jax.ShapeDtypeStruct((S, D), jnp.float32),
        scratch_shapes=[
            pltpu.VMEM((nh, ts, D), jnp.bfloat16),
            pltpu.VMEM((P, D), jnp.bfloat16),
            pltpu.VMEM((P, D), jnp.bfloat16),
            pltpu.VMEM((D, P), jnp.bfloat16),
            pltpu.VMEM((D, P), jnp.bfloat16),
            pltpu.VMEM((nf, D, tf), jnp.bfloat16),
            pltpu.VMEM((nf, D, tf), jnp.bfloat16),
            pltpu.VMEM((nf, tf, D), jnp.bfloat16),
            pltpu.SemaphoreType.DMA((nh,)),
            pltpu.SemaphoreType.DMA((nh,)),
            pltpu.SemaphoreType.DMA((2 * (P // _CB),)),
            pltpu.SemaphoreType.DMA((2 + 3 * nf,)),
            pltpu.VMEM((10, 8, P), jnp.float32),
            pltpu.VMEM((8, P), jnp.float32),
            pltpu.VMEM((nh, ts, 2 * P), jnp.float32),
            pltpu.VMEM((nh, ts, D), jnp.float32),
        ],
        compiler_params=pltpu.CompilerParams(
            dimension_semantics=("arbitrary",),
            vmem_limit_bytes=110 * 1024 * 1024,
        ),
    )(x2, A_Lambda_re, A_Lambda_im, A_log_dt, A_Dskip, gate_w,
      A_B_re, A_B_im, A_C_re, A_C_im, B_w_gate, B_w_up, B_w_down)
    return out.reshape(Bsz, S, D)
```
